```python
import os as _os
_os.environ.setdefault("JAX_PLATFORMS", "cpu")
import jax
import jax.numpy as jnp

def _softmax(x, axis=-1):
    return jax.nn.softmax(x, axis=axis)
def _gelu(x):
    return jax.nn.gelu(x, approximate=True)
def _silu(x):
    return jax.nn.silu(x)
def _sigmoid(x):
    return jax.nn.sigmoid(x)
def _layernorm(x, axis=-1, eps=1e-5):
    m = jnp.mean(x, axis=axis, keepdims=True)
    v = jnp.var(x, axis=axis, keepdims=True)
    return (x - m) / jnp.sqrt(v + eps)
def _scatter_add(tgt, idx, src, axis=0):
    return tgt.at[idx].add(src)
def _segment_sum(src, seg, n):
    return jax.ops.segment_sum(src, seg, n)
class _Rng:
    def __init__(self, key):
        self._k = key
    def _next(self):
        self._k, sub = jax.random.split(self._k)
        return sub
    def normal(self, shape):
        return jax.random.normal(self._next(), shape, dtype=jnp.bfloat16)
    def randint(self, lo, hi, shape):
        return jax.random.randint(self._next(), shape, lo, hi, dtype=jnp.int32)
    def uniform(self, shape, lo=0.0, hi=1.0):
        return jax.random.uniform(self._next(), shape, jnp.bfloat16, lo, hi)
    def permutation(self, n):
        return jax.random.permutation(self._next(), n)


kernel_name = 'gated_mix__linear_kernel_hedgehog__glu_gated_bilinear__prompt'

def setup_inputs():
    _rng = _Rng(jax.random.key(int.from_bytes(__import__("os").urandom(4), "little")))
    _w = (lambda a: (lambda t: t.astype(jnp.bfloat16) if jnp.issubdtype(t.dtype, jnp.floating) else t)(jnp.asarray(a)))
    def _A_setup():
        B, S, D, H = 1, 2048, 512, 32
        Dh = D // H
        return {
            "x": _w((lambda *s: _rng.normal(s) * 0.05)(B, S, D)),
            "wqkv": _w((lambda *s: _rng.normal(s) * 0.8)(D, 3 * D)),
            "w_phi": _w((lambda *s: _rng.normal(s) * 0.8)(H, Dh, Dh) * (Dh ** -0.5)),
            "wo": _w((lambda *s: _rng.normal(s) * 0.05)(D, D)),
        }
    _A_in = _A_setup()

    def _B_setup():
        B, S, D, F = 1, 2048, 512, 1792
        return {
            "x": _w((lambda *s: _rng.normal(s) * 0.05)(B, S, D)),
            "w_gate": _w((lambda *s: _rng.normal(s) * 1.6)(D, F) * (D ** -0.5)),
            "w_up": _w((lambda *s: _rng.normal(s) * 1.6)(D, F) * (D ** -0.5)),
            "w_down": _w((lambda *s: _rng.normal(s) * 1.6)(F, D) * (F ** -0.5)),
        }
    _B_in = _B_setup()

    return {
        "A_x": _A_in["x"],
        "A_wqkv": _A_in["wqkv"],
        "A_w_phi": _A_in["w_phi"],
        "A_wo": _A_in["wo"],
        "B_x": _B_in["x"],
        "B_w_gate": _B_in["w_gate"],
        "B_w_up": _B_in["w_up"],
        "B_w_down": _B_in["w_down"],
        "gate_w": _w((lambda *s: _rng.normal(s) * 0.05)(512) * 16.0),
    }

def reference(A_x, A_wqkv, A_w_phi, A_wo, B_x, B_w_gate, B_w_up, B_w_down, gate_w):
    def _A_ref(x, wqkv, w_phi, wo):
        B, S, D = x.shape
        H = 32; Dh = D // H
        qkv = (lambda x, *d: x.transpose(*d))((x @ wqkv).reshape(B, S, 3, H, Dh), 2, 0, 3, 1, 4)
        q, k, v = qkv[0], qkv[1], qkv[2]
        pq = jnp.einsum("bhsd,hdf->bhsf", q, w_phi)
        pk = jnp.einsum("bhsd,hdf->bhsf", k, w_phi)
        phi_q = jnp.concatenate([_softmax(pq, axis=-1), _softmax(-pq, axis=-1)], axis=-1)
        phi_k = jnp.concatenate([_softmax(pk, axis=-1), _softmax(-pk, axis=-1)], axis=-1)
        kv = jnp.einsum("bhsf,bhsd->bhfd", phi_k, v)
        z  = jnp.einsum("bhsf->bhf", phi_k)
        num = jnp.einsum("bhqf,bhfd->bhqd", phi_q, kv)
        den = jnp.einsum("bhqf,bhf->bhq", phi_q, z)[..., None] + 1e-6
        o = num / den
        return (lambda x, *d: x.transpose(*d))(o, 0, 2, 1, 3).reshape(B, S, D) @ wo

    def _B_ref(x, w_gate, w_up, w_down):
        g = jnp.einsum("bsd,df->bsf", x, w_gate)
        u = jnp.einsum("bsd,df->bsf", x, w_up)
        h = g * u
        return jnp.einsum("bsf,fd->bsd", h, w_down)

    x = A_x
    g = _sigmoid((x * gate_w).sum(-1, keepdims=True))
    a = _A_ref(x, A_wqkv, A_w_phi, A_wo)
    b = _B_ref(x, B_w_gate, B_w_up, B_w_down)
    return g * a + (1 - g) * b
```

```python
import functools

import jax
import jax.numpy as jnp
from jax import lax
import jax.experimental.pallas as pl
import jax.experimental.pallas.tpu as pltpu

F32 = jnp.float32
BF16 = jnp.bfloat16
LOG2E = 1.4426950408889634
NT = (((1,), (1,)), ((), ()))
TN = (((0,), (0,)), ((), ()))

T0 = 512
T1 = 512
FC = 256


def _dot(a, b):
    return jnp.dot(a, b, preferred_element_type=F32)


def _dg(a, b, dims):
    return lax.dot_general(a, b, dims, preferred_element_type=F32)


def _iota(shape, d):
    return lax.broadcasted_iota(jnp.int32, shape, d)


def _dual_softmax(p):
    s = [p[f * 8:(f + 1) * 8, :] for f in range(16)]
    mx, mn = s[0], s[0]
    for t in s[1:]:
        mx = jnp.maximum(mx, t)
        mn = jnp.minimum(mn, t)
    ep = [jnp.exp2(t - mx) for t in s]
    en = [jnp.exp2(mn - t) for t in s]
    zp, zn = ep[0], en[0]
    for a, b in zip(ep[1:], en[1:]):
        zp = zp + a
        zn = zn + b
    rp = 1.0 / zp
    rn = 1.0 / zn
    return [e * rp for e in ep] + [e * rn for e in en]


def _kernel(x0_ref, x1_ref, wk_ref, wv_ref, wphi_ref, gw_ref,
            wqkv_hbm, wo_hbm, wg_hbm, wu_hbm, wd_hbm,
            o_ref,
            wq_s, wo_s, wg_s, wu_s, wd_s, sems,
            a_s, wkt_s, wqt_s, wvp_s, wop_s, kv_s, z_s, l_s,
            *, n0, n1, G, D, F):
    step = pl.program_id(0)

    def copies():
        return [
            pltpu.make_async_copy(wqkv_hbm.at[:, pl.ds(0, D)], wq_s, sems.at[0]),
            pltpu.make_async_copy(wo_hbm, wo_s, sems.at[1]),
            pltpu.make_async_copy(wg_hbm, wg_s, sems.at[2]),
            pltpu.make_async_copy(wu_hbm, wu_s, sems.at[3]),
            pltpu.make_async_copy(wd_hbm, wd_s, sems.at[4]),
        ]

    def perm():
        r, c = _iota((128, 128), 0), _iota((128, 128), 1)
        return jnp.where(c == (r % 8) * 16 + r // 8, 1.0, 0.0).astype(BF16)

    @pl.when(step == 0)
    def _():
        for c in copies():
            c.start()
        e = jnp.where(_iota((128, 16), 0) // 8 == _iota((128, 16), 1), 1.0, 0.0).astype(BF16)
        r, c = _iota((128, 128), 0), _iota((128, 128), 1)
        same = (r % 8) == (c // 16)
        pm = perm()
        for g in range(G):
            sl = slice(g * 128, (g + 1) * 128)
            a = _dg(e, wphi_ref[sl, :], NT)
            a = jnp.where(same, a * LOG2E, 0.0).astype(BF16)
            a_s[g] = a
            wkt_s[sl, :] = _dg(a, wk_ref[:, sl], NT).astype(BF16)
            wvp_s[:, sl] = _dg(wv_ref[:, sl], pm, NT).astype(BF16)
        kv_s[...] = jnp.zeros_like(kv_s)
        z_s[...] = jnp.zeros_like(z_s)

    @pl.when(step < n0)
    def _():
        x = x0_ref[...]
        v = _dot(x, wvp_s[...]).astype(BF16)
        for g in range(G):
            sl = slice(g * 128, (g + 1) * 128)
            p = _dg(wkt_s[sl, :], x, NT)
            phi = jnp.concatenate(_dual_softmax(p), axis=0)
            zz = phi[:, 0:128]
            for t in range(1, T0 // 128):
                zz = zz + phi[:, t * 128:(t + 1) * 128]
            z_s[g] += zz
            kv_s[g] += _dot(phi.astype(BF16), v[:, sl])

    @pl.when(step == n0)
    def _():
        for c in copies():
            c.wait()
        pm = perm()
        m1 = (_iota((128, 256), 0) % 8) == (_iota((128, 256), 1) % 8)
        m2 = _iota((16, 256), 0) == (_iota((16, 256), 1) % 8)
        for g in range(G):
            sl = slice(g * 128, (g + 1) * 128)
            wqt_s[sl, :] = _dg(a_s[g], wq_s[:, sl], NT).astype(BF16)
            wop_s[sl, :] = _dot(pm, wo_s[sl, :]).astype(BF16)
            l_s[g, 0:128, :] = jnp.where(m1, kv_s[g].T, 0.0).astype(BF16)
            z = jnp.sum(z_s[g].T, axis=0, keepdims=True)
            l_s[g, 128:144, :] = jnp.where(m2, z, 0.0).astype(BF16)

    @pl.when(step >= n0)
    def _():
        x = x1_ref[...]
        gate = jax.nn.sigmoid(jnp.sum(x.astype(F32) * gw_ref[...].astype(F32), axis=-1, keepdims=True))
        ots = []
        for g in range(G):
            sl = slice(g * 128, (g + 1) * 128)
            p = _dg(wqt_s[sl, :], x, NT)
            phi = jnp.concatenate(_dual_softmax(p), axis=0).astype(BF16)
            nd = _dot(l_s[g], phi)
            r = 1.0 / (nd[128:136, :] + 1e-6)
            ots += [nd[d * 8:(d + 1) * 8, :] * r for d in range(16)]
        ot = jnp.concatenate(ots, axis=0).astype(BF16)
        a = _dg(ot, wop_s[...], TN)
        b = None
        for c in range(F // FC):
            cs = slice(c * FC, (c + 1) * FC)
            h = (_dot(x, wg_s[:, cs]) * _dot(x, wu_s[:, cs])).astype(BF16)
            t = _dot(h, wd_s[cs, :])
            b = t if b is None else b + t
        o_ref[...] = (gate * a + (1.0 - gate) * b).astype(o_ref.dtype)


@jax.jit
def pallas_gated_mix__linear_kernel_hedgehog__glu_gated_bilinear__prompt_kernel(
    A_x, A_wqkv, A_w_phi, A_wo, B_x, B_w_gate, B_w_up, B_w_down, gate_w,
):
    B, S, D = A_x.shape
    H, Dh, _ = A_w_phi.shape
    F = B_w_gate.shape[1]
    assert B == 1 and Dh == 16 and D % 128 == 0 and H * Dh == D
    G = D // 128
    n0, n1 = S // T0, S // T1
    x = A_x.reshape(S, D)
    any_spec = pl.BlockSpec(memory_space=pl.ANY)
    out = pl.pallas_call(
        functools.partial(_kernel, n0=n0, n1=n1, G=G, D=D, F=F),
        grid=(n0 + n1,),
        in_specs=[
            pl.BlockSpec((T0, D), lambda i: (jnp.minimum(i, n0 - 1), 0)),
            pl.BlockSpec((T1, D), lambda i: (jnp.maximum(i - n0, 0), 0)),
            pl.BlockSpec((D, D), lambda i: (0, 1)),
            pl.BlockSpec((D, D), lambda i: (0, 2)),
            pl.BlockSpec((D, Dh), lambda i: (0, 0)),
            pl.BlockSpec((1, D), lambda i: (0, 0)),
            any_spec, any_spec, any_spec, any_spec, any_spec,
        ],
        out_specs=pl.BlockSpec((T1, D), lambda i: (jnp.maximum(i - n0, 0), 0)),
        out_shape=jax.ShapeDtypeStruct((S, D), A_x.dtype),
        scratch_shapes=[
            pltpu.VMEM((D, D), BF16), pltpu.VMEM((D, D), BF16),
            pltpu.VMEM((D, F), BF16), pltpu.VMEM((D, F), BF16), pltpu.VMEM((F, D), BF16),
            pltpu.SemaphoreType.DMA((5,)),
            pltpu.VMEM((G, 128, 128), BF16),
            pltpu.VMEM((D, D), BF16), pltpu.VMEM((D, D), BF16),
            pltpu.VMEM((D, D), BF16), pltpu.VMEM((D, D), BF16),
            pltpu.VMEM((G, 256, 128), F32), pltpu.VMEM((G, 256, 128), F32),
            pltpu.VMEM((G, 144, 256), BF16),
        ],
        compiler_params=pltpu.CompilerParams(
            dimension_semantics=("arbitrary",), vmem_limit_bytes=100 * 1024 * 1024),
    )(x, x, A_wqkv, A_wqkv, A_w_phi.reshape(D, Dh), gate_w.reshape(1, D),
      A_wqkv, A_wo, B_w_gate, B_w_up, B_w_down)
    return out.reshape(B, S, D)
```

```python
import functools

import jax
import jax.numpy as jnp
from jax import lax
import jax.experimental.pallas as pl
import jax.experimental.pallas.tpu as pltpu

F32 = jnp.float32
BF16 = jnp.bfloat16
LOG2E = 1.4426950408889634
NT = (((1,), (1,)), ((), ()))
TN = (((0,), (0,)), ((), ()))

T0 = 512
T1 = 1024
TO = 256
U1 = 1
FC = 256


def _dot(a, b):
    return jnp.dot(a, b, preferred_element_type=F32)


def _dg(a, b, dims):
    return lax.dot_general(a, b, dims, preferred_element_type=F32)


def _iota(shape, d):
    return lax.broadcasted_iota(jnp.int32, shape, d)


def _dual_softmax(p):
    s = [p[f * 8:(f + 1) * 8, :] for f in range(16)]
    mx, mn = s[0], s[0]
    for t in s[1:]:
        mx = jnp.maximum(mx, t)
        mn = jnp.minimum(mn, t)
    ep = [jnp.exp2(t - mx) for t in s]
    en = [jnp.exp2(mn - t) for t in s]
    zp, zn = ep[0], en[0]
    for a, b in zip(ep[1:], en[1:]):
        zp = zp + a
        zn = zn + b
    rp = 1.0 / zp
    rn = 1.0 / zn
    return [e * rp for e in ep] + [e * rn for e in en]


def _kernel(wphi_ref, gw_ref,
            x_hbm, wqkv_hbm, wo_hbm, wg_hbm, wu_hbm, wd_hbm,
            o_hbm,
            wk_ref, o_s, osems,
            wq_s, wo_s, wg_s, wu_s, wd_s, sems, x_s, wv_s, xsems,
            a_s, wkt_s, wqt_s, wop_s, kv_s, z_s, l_s,
            *, n0, n1, G, D, F):
    step = pl.program_id(0)

    def copies():
        return [
            pltpu.make_async_copy(wqkv_hbm.at[:, pl.ds(0, D)], wq_s, sems.at[0]),
            pltpu.make_async_copy(wo_hbm, wo_s, sems.at[1]),
            pltpu.make_async_copy(wg_hbm, wg_s, sems.at[2]),
            pltpu.make_async_copy(wu_hbm, wu_s, sems.at[3]),
            pltpu.make_async_copy(wd_hbm, wd_s, sems.at[4]),
        ]

    def xcopy(i):
        rows = pl.ds(pl.multiple_of(i * T0, T0), T0)
        return pltpu.make_async_copy(x_hbm.at[rows, :], x_s.at[rows, :], xsems.at[i])

    wv_copy = pltpu.make_async_copy(wqkv_hbm.at[:, pl.ds(2 * D, D)], wv_s, sems.at[5])

    def perm():
        r, c = _iota((128, 128), 0), _iota((128, 128), 1)
        return jnp.where(c == (r % 8) * 16 + r // 8, 1.0, 0.0).astype(BF16)

    @pl.when(step == 0)
    def _():
        wk_copy = pltpu.make_async_copy(wqkv_hbm.at[:, pl.ds(D, D)], wk_ref, sems.at[6])
        wk_copy.start()
        xcopy(0).start()
        wv_copy.start()
        w = wphi_ref[...]
        u_keep = (_iota((128, 256), 0) // 8) == (_iota((128, 256), 1) % 16)
        cm = jnp.where(_iota((256, 128), 0) // 16 == _iota((256, 128), 1) % 16, 1.0, 0.0).astype(BF16)
        r, c = _iota((128, 128), 0), _iota((128, 128), 1)
        same = (r % 8) == (c // 16)
        for g in range(G):
            sl = slice(g * 128, (g + 1) * 128)
            sel = jnp.where(_iota((128, 32), 0) % 8 + g * 8 == _iota((128, 32), 1), 1.0, 0.0)
            u = jnp.where(u_keep, _dg(sel.astype(BF16), w, NT), 0.0).astype(BF16)
            a = _dot(u, cm)
            a = jnp.where(same, a * LOG2E, 0.0).astype(BF16)
            a_s[g] = a
        kv_s[...] = jnp.zeros_like(kv_s)
        z_s[...] = jnp.zeros_like(z_s)
        wk_copy.wait()
        for g in range(G):
            sl = slice(g * 128, (g + 1) * 128)
            wkt_s[sl, :] = _dg(a_s[g], wk_ref[:, sl], NT).astype(BF16)
        wv_copy.wait()
        for i in range(1, n0):
            xcopy(i).start()

    @pl.when(step < n0)
    def _():
        xcopy(step).wait()

        @pl.when(step == min(1, n0 - 1))
        def _():
            for c in copies():
                c.start()

        x = x_s[pl.ds(pl.multiple_of(step * T0, T0), T0), :]
        pa = _dg(wkt_s[...], x, NT)
        v = _dot(x, wv_s[...]).astype(BF16)
        for g in range(G):
            sl = slice(g * 128, (g + 1) * 128)
            p = pa[sl, :]
            phi = jnp.concatenate(_dual_softmax(p), axis=0)
            zz = phi[:, 0:128]
            for t in range(1, T0 // 128):
                zz = zz + phi[:, t * 128:(t + 1) * 128]
            z_s[g] += zz
            kv_s[g] += _dot(phi.astype(BF16), v[:, sl])

    @pl.when(step == n0)
    def _():
        for c in copies():
            c.wait()
        pm = perm()
        m1 = (_iota((128, 256), 0) % 8) == (_iota((128, 256), 1) % 8)
        m2 = _iota((16, 256), 0) == (_iota((16, 256), 1) % 8)
        for g in range(G):
            sl = slice(g * 128, (g + 1) * 128)
            wqt_s[sl, :] = _dg(a_s[g], wq_s[:, sl], NT).astype(BF16)
            wop_s[sl, :] = _dot(pm, wo_s[sl, :]).astype(BF16)
            l_s[g, 0:128, :] = jnp.where(
                m1, _dg(pm, kv_s[g].astype(BF16), NT), 0.0).astype(BF16)
            z = jnp.sum(z_s[g].T, axis=0, keepdims=True)
            l_s[g, 128:144, :] = jnp.where(m2, z, 0.0).astype(BF16)

    def ocopy(i):
        rows = pl.ds(pl.multiple_of(i * TO, TO), TO)
        return pltpu.make_async_copy(o_s.at[rows, :], o_hbm.at[rows, :], osems.at[i])

    def tile(i):
        rows = pl.ds(pl.multiple_of(i * T1, T1), T1)
        x = x_s[rows, :]
        gate = jax.nn.sigmoid(jnp.sum(x.astype(F32) * gw_ref[...].astype(F32).reshape(1, D), axis=-1, keepdims=True))
        ots = []
        for g in range(G):
            sl = slice(g * 128, (g + 1) * 128)
            p = _dg(wqt_s[sl, :], x, NT)
            phi = jnp.concatenate(_dual_softmax(p), axis=0).astype(BF16)
            nd = _dot(l_s[g], phi)
            r = 1.0 / (nd[128:136, :] + 1e-6)
            ots += [nd[d * 8:(d + 1) * 8, :] * r for d in range(16)]
        ot = jnp.concatenate(ots, axis=0).astype(BF16)
        h = jnp.concatenate([
            (_dot(x, wg_s[:, c:c + FC]) * _dot(x, wu_s[:, c:c + FC])).astype(BF16)
            for c in range(0, F, FC)], axis=1)
        for j in range(T1 // TO):
            rs = slice(j * TO, (j + 1) * TO)
            a = _dg(ot[:, rs], wop_s[...], TN)
            b = _dot(h[rs], wd_s[...])
            k = i * (T1 // TO) + j
            o_s[pl.ds(pl.multiple_of(k * TO, TO), TO), :] = (
                gate[rs] * a + (1.0 - gate[rs]) * b).astype(o_s.dtype)
            ocopy(k).start()

    @pl.when(step >= n0)
    def _():
        for j in range(U1):
            tile((step - n0) * U1 + j)

    @pl.when(step == n0 + n1 - 1)
    def _():
        for i in range(n1 * U1 * T1 // TO):
            ocopy(i).wait()


@jax.jit
def pallas_gated_mix__linear_kernel_hedgehog__glu_gated_bilinear__prompt_kernel(
    A_x, A_wqkv, A_w_phi, A_wo, B_x, B_w_gate, B_w_up, B_w_down, gate_w,
):
    B, S, D = A_x.shape
    H, Dh, _ = A_w_phi.shape
    F = B_w_gate.shape[1]
    assert B == 1 and Dh == 16 and D % 128 == 0 and H == 32 and H * Dh == D
    G = D // 128
    n0, n1 = S // T0, S // (T1 * U1)
    x = A_x.reshape(S, D)
    any_spec = pl.BlockSpec(memory_space=pl.ANY)
    out = pl.pallas_call(
        functools.partial(_kernel, n0=n0, n1=n1, G=G, D=D, F=F),
        grid=(n0 + n1,),
        in_specs=[
            pl.BlockSpec((Dh * Dh, H), lambda i: (0, 0)),
            pl.BlockSpec((D,), lambda i: (0,)),
            any_spec, any_spec, any_spec, any_spec, any_spec, any_spec,
        ],
        out_specs=any_spec,
        out_shape=jax.ShapeDtypeStruct((S, D), A_x.dtype),
        scratch_shapes=[
            pltpu.VMEM((D, D), BF16),
            pltpu.VMEM((S, D), A_x.dtype), pltpu.SemaphoreType.DMA((S // TO,)),
            pltpu.VMEM((D, D), BF16), pltpu.VMEM((D, D), BF16),
            pltpu.VMEM((D, F), BF16), pltpu.VMEM((D, F), BF16), pltpu.VMEM((F, D), BF16),
            pltpu.SemaphoreType.DMA((7,)),
            pltpu.VMEM((S, D), BF16), pltpu.VMEM((D, D), BF16),
            pltpu.SemaphoreType.DMA((n0,)),
            pltpu.VMEM((G, 128, 128), BF16),
            pltpu.VMEM((D, D), BF16), pltpu.VMEM((D, D), BF16),
            pltpu.VMEM((D, D), BF16),
            pltpu.VMEM((G, 256, 128), F32), pltpu.VMEM((G, 256, 128), F32),
            pltpu.VMEM((G, 144, 256), BF16),
        ],
        compiler_params=pltpu.CompilerParams(
            dimension_semantics=("arbitrary",), vmem_limit_bytes=100 * 1024 * 1024),
    )(A_w_phi.transpose(1, 2, 0).reshape(Dh * Dh, H), gate_w,
      x, A_wqkv, A_wo, B_w_gate, B_w_up, B_w_down)
    return out.reshape(B, S, D)
```
